```python
import os as _os
_os.environ.setdefault("JAX_PLATFORMS", "cpu")
import jax
import jax.numpy as jnp

def _softmax(x, axis=-1):
    return jax.nn.softmax(x, axis=axis)
def _gelu(x):
    return jax.nn.gelu(x, approximate=True)
def _silu(x):
    return jax.nn.silu(x)
def _sigmoid(x):
    return jax.nn.sigmoid(x)
def _layernorm(x, axis=-1, eps=1e-5):
    m = jnp.mean(x, axis=axis, keepdims=True)
    v = jnp.var(x, axis=axis, keepdims=True)
    return (x - m) / jnp.sqrt(v + eps)
def _scatter_add(tgt, idx, src, axis=0):
    return tgt.at[idx].add(src)
def _segment_sum(src, seg, n):
    return jax.ops.segment_sum(src, seg, n)
class _Rng:
    def __init__(self, key):
        self._k = key
    def _next(self):
        self._k, sub = jax.random.split(self._k)
        return sub
    def normal(self, shape):
        return jax.random.normal(self._next(), shape, dtype=jnp.bfloat16)
    def randint(self, lo, hi, shape):
        return jax.random.randint(self._next(), shape, lo, hi, dtype=jnp.int32)
    def uniform(self, shape, lo=0.0, hi=1.0):
        return jax.random.uniform(self._next(), shape, jnp.bfloat16, lo, hi)
    def permutation(self, n):
        return jax.random.permutation(self._next(), n)


kernel_name = 'standalone__mha_block_cached__near_ridge'

def setup_inputs():
    _rng = _Rng(jax.random.key(int.from_bytes(__import__("os").urandom(4), "little")))
    _w = (lambda a: (lambda t: t.astype(jnp.bfloat16) if jnp.issubdtype(t.dtype, jnp.floating) else t)(jnp.asarray(a)))
    B, Sq, D = 8, 112, 640
    H, Sk, Dh = 32, 512, 192
    return {
        "x": _w((lambda *s: _rng.normal(s) * 0.8)(B, Sq, D)),
        "k_cache": _w((lambda *s: _rng.normal(s) * 0.8)(B, H, Sk, Dh)),
        "v_cache": _w((lambda *s: _rng.normal(s) * 0.05)(B, H, Sk, Dh)),
        "wq": _w((lambda *s: _rng.normal(s) * 0.8)(D, H * Dh) * (D ** -0.5)),
        "wo": _w((lambda *s: _rng.normal(s) * 0.05)(H * Dh, D) * ((H * Dh) ** -0.5)),
    }

def reference(x, k_cache, v_cache, wq, wo):
    B, Sq, D = x.shape
    H, Dh = 32, 192
    q = (lambda x, *d: x.transpose(*d))((x @ wq).reshape(B, Sq, H, Dh), 0, 2, 1, 3)
    scores = jnp.einsum("bhqd,bhkd->bhqk", q, k_cache) * (Dh ** -0.5)
    p = _softmax(scores, axis=-1)
    o = jnp.einsum("bhqk,bhkd->bhqd", p, v_cache)
    return (lambda x, *d: x.transpose(*d))(o, 0, 2, 1, 3).reshape(B, Sq, H * Dh) @ wo
```

```python
import functools, math
import jax, jax.numpy as jnp
from jax import lax
from jax.experimental import pallas as pl
from jax.experimental.pallas import tpu as pltpu

B, SQ, D = 8, 112, 640
H, SK, DH = 32, 512, 192
HP = H // 2
PW = 2 * DH
NU = B * HP
SCALE = (DH ** -0.5) * math.log2(math.e)
BF = jnp.bfloat16
F32 = jnp.float32

def nn(a, b): return lax.dot_general(a, b, (((1,), (0,)), ((), ())), preferred_element_type=F32)
def nt(a, b): return lax.dot_general(a, b, (((1,), (1,)), ((), ())), preferred_element_type=F32)
def tn(a, b): return lax.dot_general(a, b, (((0,), (0,)), ((), ())), preferred_element_type=F32)

def softmax_parts(s, normalize):
    m = jnp.max(s, axis=-1, keepdims=True)
    p = jnp.exp2(s - m)
    l = jnp.sum(p, axis=-1, keepdims=True)
    r = 1.0 / l
    if normalize:
        return (p * r).astype(BF), None
    return p.astype(BF), r

def _build(G=4, form='B', NSB=4, LAB=2, no_dma=False, no_compute=False, nbc=True):
    NBLK = NU // G
    BPH = B // G
    LBPH = int(math.log2(BPH))
    assert NSB & (NSB - 1) == 0 and LAB < NSB

    def kernel(x_hbm, wq_hbm, kt_hbm, vt_hbm, wo_hbm, o_hbm,
               x_s, wq_s, wo_s, k_s, v_s, q_s, o_s, acc_s, out_s,
               sem_x, sem_wq, sem_wo, sem_k, sem_v, sem_o):
        j = pl.program_id(0)

        def blk(jb):
            hp = jb >> LBPH if not isinstance(jb, int) else jb // BPH
            g = jb & (BPH - 1)
            return hp, g, jb & (NSB - 1)
        def k_copy(jb):
            hp, g, s = blk(jb)
            return pltpu.make_async_copy(kt_hbm.at[pl.ds(g * G, G), hp], k_s.at[s], sem_k.at[s])
        def v_copy(jb):
            hp, g, s = blk(jb)
            return pltpu.make_async_copy(vt_hbm.at[pl.ds(g * G, G), hp], v_s.at[s], sem_v.at[s])
        def wq_copy(hp):
            off = hp * PW if isinstance(hp, int) else pl.multiple_of(hp * PW, 128)
            return pltpu.make_async_copy(wq_hbm.at[:, pl.ds(off, PW)], wq_s.at[hp], sem_wq.at[hp])
        def wo_copy(hp):
            off = hp * PW if isinstance(hp, int) else pl.multiple_of(hp * PW, 128)
            return pltpu.make_async_copy(wo_hbm.at[pl.ds(off, PW), :], wo_s.at[hp], sem_wo.at[hp])
        x_copy = lambda: pltpu.make_async_copy(x_hbm, x_s, sem_x.at[0])

        def qproj(hp, b):
            xv = x_s[pl.ds(pl.multiple_of(b * SQ, 16), SQ), :]
            q = nn(xv, wq_s[hp]) * SCALE
            lane = lax.broadcasted_iota(jnp.int32, (SQ, 128), 1)
            mid = q[:, 128:256]
            qe = jnp.concatenate([q[:, 0:128], jnp.where(lane < 64, mid, 0.0)], axis=1).astype(BF)
            qo = jnp.concatenate([jnp.where(lane >= 64, mid, 0.0), q[:, 256:384]], axis=1).astype(BF)
            return qe, qo

        def scores(qe, qo, s, i):
            se = nn(qe, k_s[s, i, 0:256, :])
            so = nn(qo, k_s[s, i, 128:384, :])
            return se, so

        def pv(se, so, s, i):
            if form == 'A':
                pe, re = softmax_parts(se, False)
                po, ro = softmax_parts(so, False)
                oe = nt(pe, v_s[s, i, 0:256, :]) * re
                oo = nt(po, v_s[s, i, 128:384, :]) * ro
                lane = lax.broadcasted_iota(jnp.int32, (SQ, 128), 1)
                return jnp.concatenate([oe[:, 0:128], jnp.where(lane < 64, oe[:, 128:256], oo[:, 0:128]), oo[:, 128:256]], axis=1).astype(BF)
            else:
                pe, _ = softmax_parts(se, True)
                po, _ = softmax_parts(so, True)
                oet = nt(v_s[s, i, 0:192, :], pe)
                oot = nt(v_s[s, i, 192:384, :], po)
                return jnp.concatenate([oet, oot], axis=0).astype(BF)

        def outproj(o, hp, b):
            rows = pl.ds(pl.multiple_of(b * SQ, 16), SQ)
            y = nn(o, wo_s[hp]) if form == 'A' else tn(o, wo_s[hp])
            acc_s[rows, :] += y

        @pl.when(j == 0)
        def _():
            if not no_dma:
                x_copy().start()
                wq_copy(0).start()
                k_copy(0).start(); v_copy(0).start()
                wo_copy(0).start()
                for jb in range(1, LAB):
                    k_copy(jb).start(); v_copy(jb).start()
            acc_s[...] = jnp.zeros_like(acc_s)
            o_s[...] = jnp.zeros_like(o_s)
            if not no_dma:
                x_copy().wait()
                wq_copy(0).wait()
            qe, qo = qproj(0, 0)
            q_s[0] = qe
            q_s[1] = qo

        hp = j >> LBPH
        g = j & (BPH - 1)
        s = j & (NSB - 1)
        if not no_dma:
            @pl.when(jnp.logical_and(g == 0, hp + 1 < HP))
            def _():
                wq_copy(hp + 1).start()
                wo_copy(hp + 1).start()
            @pl.when(j + LAB < NBLK)
            def _():
                k_copy(j + LAB).start(); v_copy(j + LAB).start()
            @pl.when(g == 0)
            def _():
                wo_copy(hp).wait()
            @pl.when(jnp.logical_and(g == BPH - 1, hp + 1 < HP))
            def _():
                wq_copy(hp + 1).wait()
            k_copy(j).wait()
            v_copy(j).wait()

        if not no_compute:
            qe, qo = q_s[0], q_s[1]
            o_prev = o_s[...]
            for i in range(G):
                b = g * G + i
                se, so = scores(qe, qo, s, i)
                if i == 0:
                    bp = (b + (B - 1)) & (B - 1)
                    hpp = jnp.maximum(jnp.where(g == 0, hp - 1, hp), 0)
                else:
                    bp, hpp = b - 1, hp
                outproj(o_prev, hpp, bp)
                if i == G - 1:
                    bn = (b + 1) & (B - 1)
                    hpn = jnp.minimum(jnp.where(g == BPH - 1, hp + 1, hp), HP - 1)
                else:
                    bn, hpn = b + 1, hp
                qe, qo = qproj(hpn, bn)
                o_prev = pv(se, so, s, i)
            q_s[0] = qe
            q_s[1] = qo
            o_s[...] = o_prev

        @pl.when(j == NBLK - 1)
        def _():
            outproj(o_s[...], HP - 1, B - 1)
            out_s[...] = acc_s[...].astype(BF)
            cp = pltpu.make_async_copy(out_s, o_hbm, sem_o.at[0])
            cp.start()
            cp.wait()

    def f(x, k_cache, v_cache, wq, wo):
        kt = jnp.transpose(k_cache, (0, 1, 3, 2)).reshape(B, HP, PW, SK)
        vt = jnp.transpose(v_cache, (0, 1, 3, 2)).reshape(B, HP, PW, SK)
        x2 = x.reshape(B * SQ, D)
        anyspec = pl.BlockSpec(memory_space=pl.ANY)
        o_shape = (SQ, PW) if form == 'A' else (PW, SQ)
        out = pl.pallas_call(
            kernel,
            grid=(NBLK,),
            in_specs=[anyspec] * 5,
            out_specs=anyspec,
            out_shape=jax.ShapeDtypeStruct((B * SQ, D), BF),
            scratch_shapes=[
                pltpu.VMEM((B * SQ, D), BF),
                pltpu.VMEM((HP, D, PW), BF),
                pltpu.VMEM((HP, PW, D), BF),
                pltpu.VMEM((NSB, G, PW, SK), BF),
                pltpu.VMEM((NSB, G, PW, SK), BF),
                pltpu.VMEM((2, SQ, 256), BF),
                pltpu.VMEM(o_shape, BF),
                pltpu.VMEM((B * SQ, D), F32),
                pltpu.VMEM((B * SQ, D), BF),
                pltpu.SemaphoreType.DMA((1,)),
                pltpu.SemaphoreType.DMA((HP,)),
                pltpu.SemaphoreType.DMA((HP,)),
                pltpu.SemaphoreType.DMA((NSB,)),
                pltpu.SemaphoreType.DMA((NSB,)),
                pltpu.SemaphoreType.DMA((1,)),
            ],
            compiler_params=pltpu.CompilerParams(
                dimension_semantics=("arbitrary",),
                disable_bounds_checks=nbc,
                vmem_limit_bytes=110 * 1024 * 1024),
        )(x2, wq, kt, vt, wo)
        return out.reshape(B, SQ, D)
    return f


_F = _build()


@jax.jit
def pallas_standalone__mha_block_cached__near_ridge_kernel(x, k_cache, v_cache, wq, wo):
    return _F(x, k_cache, v_cache, wq, wo)
```

```python
import functools
import math

import jax
import jax.numpy as jnp
from jax import lax
from jax.experimental import pallas as pl
from jax.experimental.pallas import tpu as pltpu

B, SQ, D = 8, 112, 640
H, SK, DH = 32, 512, 192
HP = H // 2
PW = 2 * DH
NU = B * HP
NH = NU // 2
SCALE = (DH ** -0.5) * math.log2(math.e)
BF = jnp.bfloat16
F32 = jnp.float32

LB = 7
NR = 8
LA = 4
NSPLIT = 4
QR = 8
NAB = 2 * HP - LB
H0 = 2 * NAB
NWQ0 = (LB - 1) // 2 + 2


def _nn(a, b):
    return lax.dot_general(a, b, (((1,), (0,)), ((), ())), preferred_element_type=F32)


def _nt(a, b):
    return lax.dot_general(a, b, (((1,), (1,)), ((), ())), preferred_element_type=F32)


def _tn(a, b):
    return lax.dot_general(a, b, (((0,), (0,)), ((), ())), preferred_element_type=F32)


def _softmax(s):
    m = jnp.max(s, axis=-1, keepdims=True)
    p = jnp.exp2(s - m)
    l = jnp.sum(p, axis=-1, keepdims=True)
    return (p * (1.0 / l)).astype(BF)


def _kernel(x_hbm, wq_hbm, kt_hbm, vt_hbm, wo_hbm, o_hbm,
            x_s, wq_s, wo_s, k_s, v_s, q_s, o_s, acc_s, out_s,
            sem_x, sem_wq, sem_wo, sem_k, sem_v, sem_o, sem_f):

    def k_copy(h):
        slot = h & (NR - 1)
        return pltpu.make_async_copy(
            kt_hbm.at[pl.ds((h & 3) * 2, 2), h >> 2], k_s.at[slot], sem_k.at[slot])

    def v_copy(h):
        slot = h & (NR - 1)
        return pltpu.make_async_copy(
            vt_hbm.at[pl.ds((h & 3) * 2, 2), h >> 2], v_s.at[slot], sem_v.at[slot])

    def kv_start(h):
        k_copy(h).start()
        v_copy(h).start()

    def kv_wait(h):
        k_copy(h).wait()
        v_copy(h).wait()

    def w_off(hp):
        return hp * PW if isinstance(hp, int) else pl.multiple_of(hp * PW, 128)

    def wq_copy(hp):
        return pltpu.make_async_copy(
            wq_hbm.at[:, pl.ds(w_off(hp), PW)], wq_s.at[hp], sem_wq.at[hp & 7])

    def wo_copy(hp):
        return pltpu.make_async_copy(
            wo_hbm.at[pl.ds(w_off(hp), PW), :], wo_s.at[hp], sem_wo.at[hp & 1])

    def rows_of(b, n=1):
        if isinstance(b, int):
            return pl.ds(b * SQ, n * SQ)
        return pl.ds(pl.multiple_of(b * SQ, 16), n * SQ)

    def x_copy(half):
        r = rows_of(half * 4, 4)
        return pltpu.make_async_copy(x_hbm.at[r], x_s.at[r], sem_x.at[half])

    def out_copy(b0, nb, k):
        r = rows_of(b0, nb)
        return pltpu.make_async_copy(out_s.at[r], o_hbm.at[r], sem_o.at[k])

    def fence():
        pl.semaphore_signal(sem_f, 1)
        pl.semaphore_wait(sem_f, 1)

    def qproj(hp, b, n=1):
        q = _nn(x_s[rows_of(b, n), :], wq_s[hp]) * SCALE
        lane = lax.broadcasted_iota(jnp.int32, (n * SQ, 128), 1)
        mid = q[:, 128:256]
        qe = jnp.concatenate([q[:, 0:128], jnp.where(lane < 64, mid, 0.0)], axis=1)
        qo = jnp.concatenate([jnp.where(lane >= 64, mid, 0.0), q[:, 256:384]], axis=1)
        qs = hp & (QR - 1)
        q_s[qs, 0, rows_of(b, n), :] = qe.astype(BF)
        q_s[qs, 1, rows_of(b, n), :] = qo.astype(BF)

    def scores(hp, b, s, i):
        qs = hp & (QR - 1)
        se = _nn(q_s[qs, 0, rows_of(b), :], k_s[s, i, 0:256, :])
        so = _nn(q_s[qs, 1, rows_of(b), :], k_s[s, i, 128:384, :])
        return se, so

    def pv_p(pe, po, s, i):
        oet = _nt(v_s[s, i, 0:192, :], pe)
        oot = _nt(v_s[s, i, 192:384, :], po)
        return jnp.concatenate([oet, oot], axis=0).astype(BF)

    def pv(se, so, s, i):
        return pv_p(_softmax(se), _softmax(so), s, i)

    def outproj(o, hp, b, emit=False):
        r = acc_s[rows_of(b), :] + _tn(o, wo_s[hp])
        acc_s[rows_of(b), :] = r
        if emit:
            out_s[rows_of(b), :] = r.astype(BF)

    seq = [x_copy(0), wq_copy(0), x_copy(1)]
    seq += [wq_copy(hp) for hp in range(1, NWQ0 - 1)]
    jstar = 2 * (NWQ0 - 1) - LB
    if jstar == 0:
        seq += [wq_copy(NWQ0 - 1)]
    seq += [wo_copy(0)]
    for h in range(LA):
        if h == 2 and jstar == 1:
            seq += [wq_copy(NWQ0 - 1)]
        seq += [k_copy(h), v_copy(h)]
    for c in seq:
        c.start()
        fence()
    acc_s[...] = jnp.zeros_like(acc_s)
    o_s[...] = jnp.zeros_like(o_s)

    def pro_body(it, c):
        hp = it >> 1
        half = it & 1

        @pl.when(it < 2)
        def _():
            x_copy(half).wait()

        @pl.when(half == 0)
        def _():
            wq_copy(hp).wait()

        qproj(hp, half * 4, 4)
        return c

    lax.fori_loop(0, LB, pro_body, 0)

    def a_body(j, c):
        hp = j >> 1
        g = j & 1
        h0 = 2 * j
        jq = j + LB
        hpq = jq >> 1
        gq = jq & 1

        @pl.when(gq == 0)
        def _():
            wq_copy(hpq).wait()

        @pl.when(g == 0)
        def _():
            wo_copy(hp).wait()

        kv_wait(h0)
        kv_wait(h0 + 1)

        @pl.when(jnp.logical_and(gq == 0, hpq + 1 < HP))
        def _():
            wq_copy(hpq + 1).start()

        @pl.when(g == 0)
        def _():
            wo_copy(hp + 1).start()

        kv_start(h0 + LA)
        kv_start(h0 + LA + 1)

        o_prev = o_s[...]
        for i in range(4):
            b = g * 4 + i
            s = (h0 + i // 2) & (NR - 1)
            se, so = scores(hp, b, s, i % 2)
            if i == 0:
                bp = (b + (B - 1)) & (B - 1)
                hpp = jnp.maximum(hp - 1 + g, 0)
            else:
                bp, hpp = b - 1, hp
            outproj(o_prev, hpp, bp)
            qproj(hpq, gq * 4 + i)
            o_prev = pv(se, so, s, i % 2)
        o_s[...] = o_prev
        return c

    lax.fori_loop(0, NAB, a_body, 0)

    def n_body(h, c, last=False, split=False):
        hp = h >> 2
        q4 = h & 3
        b0 = q4 * 2
        s = h & (NR - 1)
        if not last:
            @pl.when(q4 == 0)
            def _():
                wo_copy(hp).wait()
        if split:
            k_copy(h).wait()
        else:
            kv_wait(h)
        if not last:
            @pl.when(jnp.logical_and(q4 == 0, hp + 1 < HP))
            def _():
                wo_copy(hp + 1).start()

            @pl.when(h + LA < NH)
            def _():
                kv_start(h + LA)

        o_prev = o_s[...]
        se0, so0 = scores(hp, b0, s, 0)
        se1, so1 = scores(hp, b0 + 1, s, 1)
        if isinstance(h, int):
            bp = (b0 + B - 1) % B
            hpp = hp - 1 if q4 == 0 else hp
        else:
            bp = (b0 + (B - 1)) & (B - 1)
            hpp = jnp.where(q4 == 0, hp - 1, hp)
        outproj(o_prev, hpp, bp, emit=True)
        if split:
            p0 = (_softmax(se0), _softmax(so0))
            p1 = (_softmax(se1), _softmax(so1))
            v_copy(h).wait()
            if last:
                out_copy(0, 6, 0).start()
            o0 = pv_p(*p0, s, 0)
            o1 = pv_p(*p1, s, 1)
        else:
            o0 = pv(se0, so0, s, 0)
            o1 = pv(se1, so1, s, 1)
        outproj(o0, hp, b0, emit=True)
        if last:
            out_copy(6, 1, 1).start()
            outproj(o1, hp, b0 + 1, emit=True)
            out_copy(7, 1, 2).start()
        else:
            o_s[...] = o1
        return c

    lax.fori_loop(H0, NH - NSPLIT, n_body, 0)
    lax.fori_loop(NH - NSPLIT, NH - 1, functools.partial(n_body, split=True), 0)
    n_body(NH - 1, 0, last=True, split=True)
    out_copy(0, 6, 0).wait()
    out_copy(6, 1, 1).wait()
    out_copy(7, 1, 2).wait()


@jax.jit
def pallas_standalone__mha_block_cached__near_ridge_kernel(
    x: jax.Array,
    k_cache: jax.Array,
    v_cache: jax.Array,
    wq: jax.Array,
    wo: jax.Array,
):
    kt = jnp.transpose(k_cache, (0, 1, 3, 2)).reshape(B, HP, PW, SK)
    vt = jnp.transpose(v_cache, (0, 1, 3, 2)).reshape(B, HP, PW, SK)
    x2 = x.reshape(B * SQ, D)
    anyspec = pl.BlockSpec(memory_space=pl.ANY)
    out = pl.pallas_call(
        _kernel,
        in_specs=[anyspec] * 5,
        out_specs=anyspec,
        out_shape=jax.ShapeDtypeStruct((B * SQ, D), BF),
        scratch_shapes=[
            pltpu.VMEM((B * SQ, D), BF),
            pltpu.VMEM((HP, D, PW), BF),
            pltpu.VMEM((HP, PW, D), BF),
            pltpu.VMEM((NR, 2, PW, SK), BF),
            pltpu.VMEM((NR, 2, PW, SK), BF),
            pltpu.VMEM((QR, 2, B * SQ, 256), BF),
            pltpu.VMEM((PW, SQ), BF),
            pltpu.VMEM((B * SQ, D), F32),
            pltpu.VMEM((B * SQ, D), BF),
            pltpu.SemaphoreType.DMA((2,)),
            pltpu.SemaphoreType.DMA((8,)),
            pltpu.SemaphoreType.DMA((2,)),
            pltpu.SemaphoreType.DMA((NR,)),
            pltpu.SemaphoreType.DMA((NR,)),
            pltpu.SemaphoreType.DMA((3,)),
            pltpu.SemaphoreType.REGULAR,
        ],
        compiler_params=pltpu.CompilerParams(
            disable_bounds_checks=True,
            disable_semaphore_checks=True,
            vmem_limit_bytes=100 * 1024 * 1024),
    )(x2, wq, kt, vt, wo)
    return out.reshape(B, SQ, D)
```

```python
import functools
import math

import jax
import jax.numpy as jnp
from jax import lax
from jax.experimental import pallas as pl
from jax.experimental.pallas import tpu as pltpu

B, SQ, D = 8, 112, 640
H, SK, DH = 32, 512, 192
HP = H // 2
PW = 2 * DH
NU = B * HP
NH = NU // 2
SCALE = (DH ** -0.5) * math.log2(math.e)
BF = jnp.bfloat16
F32 = jnp.float32

LB = 7
NR = 8
LA = 4
NSPLIT = 4
QR = 8
NAB = 2 * HP - LB
H0 = 2 * NAB
NWQ0 = (LB - 1) // 2 + 2


def _nn(a, b):
    return lax.dot_general(a, b, (((1,), (0,)), ((), ())), preferred_element_type=F32)


def _nt(a, b):
    return lax.dot_general(a, b, (((1,), (1,)), ((), ())), preferred_element_type=F32)


def _tn(a, b):
    return lax.dot_general(a, b, (((0,), (0,)), ((), ())), preferred_element_type=F32)


def _softmax(s):
    m = jnp.max(s, axis=-1, keepdims=True)
    p = jnp.exp2(s - m)
    l = jnp.sum(p, axis=-1, keepdims=True)
    return (p * (1.0 / l)).astype(BF)


def _kernel(x_hbm, wq_hbm, kt_hbm, vt_hbm, wo_hbm, o_hbm,
            x_s, wq_s, wo_s, k_s, v_s, q_s, o_s, acc_s, out_s,
            sem_x, sem_wq, sem_wo, sem_k, sem_v, sem_o, sem_f):

    def k_copy(h):
        slot = h & (NR - 1)
        return pltpu.make_async_copy(
            kt_hbm.at[pl.ds((h & 3) * 2, 2), h >> 2], k_s.at[slot], sem_k.at[slot])

    def v_copy(h):
        slot = h & (NR - 1)
        return pltpu.make_async_copy(
            vt_hbm.at[pl.ds((h & 3) * 2, 2), h >> 2], v_s.at[slot], sem_v.at[slot])

    def kv_start(h):
        k_copy(h).start()
        v_copy(h).start()

    def kv_wait(h):
        k_copy(h).wait()
        v_copy(h).wait()

    def w_off(hp):
        return hp * PW if isinstance(hp, int) else pl.multiple_of(hp * PW, 128)

    def wq_copy(hp):
        return pltpu.make_async_copy(
            wq_hbm.at[:, pl.ds(w_off(hp), PW)], wq_s.at[hp], sem_wq.at[hp & 7])

    def wo_copy(hp):
        return pltpu.make_async_copy(
            wo_hbm.at[pl.ds(w_off(hp), PW), :], wo_s.at[hp], sem_wo.at[hp & 1])

    def rows_of(b, n=1):
        if isinstance(b, int):
            return pl.ds(b * SQ, n * SQ)
        return pl.ds(pl.multiple_of(b * SQ, 16), n * SQ)

    def x_copy(half):
        r = rows_of(half * 4, 4)
        return pltpu.make_async_copy(x_hbm.at[r], x_s.at[r], sem_x.at[half])

    def out_copy(b0, nb, k):
        r = rows_of(b0, nb)
        return pltpu.make_async_copy(out_s.at[r], o_hbm.at[r], sem_o.at[k])

    def fence():
        pl.semaphore_signal(sem_f, 1)
        pl.semaphore_wait(sem_f, 1)

    def qproj(hp, b, n=1):
        q = _nn(x_s[rows_of(b, n), :], wq_s[hp]) * SCALE
        lane = lax.broadcasted_iota(jnp.int32, (n * SQ, 128), 1)
        mid = q[:, 128:256]
        qe = jnp.concatenate([q[:, 0:128], jnp.where(lane < 64, mid, 0.0)], axis=1)
        qo = jnp.concatenate([jnp.where(lane >= 64, mid, 0.0), q[:, 256:384]], axis=1)
        qs = hp & (QR - 1)
        q_s[qs, 0, rows_of(b, n), :] = qe.astype(BF)
        q_s[qs, 1, rows_of(b, n), :] = qo.astype(BF)

    def scores(hp, b, s, i):
        qs = hp & (QR - 1)
        se = _nn(q_s[qs, 0, rows_of(b), :], k_s[s, i, 0:256, :])
        so = _nn(q_s[qs, 1, rows_of(b), :], k_s[s, i, 128:384, :])
        return se, so

    def pv_p(pe, po, s, i):
        oet = _nt(v_s[s, i, 0:192, :], pe)
        oot = _nt(v_s[s, i, 192:384, :], po)
        return jnp.concatenate([oet, oot], axis=0).astype(BF)

    def pv(se, so, s, i):
        return pv_p(_softmax(se), _softmax(so), s, i)

    def outproj(o, hp, b, emit=False):
        r = acc_s[rows_of(b), :] + _tn(o, wo_s[hp])
        acc_s[rows_of(b), :] = r
        if emit:
            out_s[rows_of(b), :] = r.astype(BF)

    seq = [x_copy(0), wq_copy(0), x_copy(1)]
    seq += [wq_copy(hp) for hp in range(1, NWQ0 - 1)]
    jstar = 2 * (NWQ0 - 1) - LB
    if jstar == 0:
        seq += [wq_copy(NWQ0 - 1)]
    seq += [wo_copy(0)]
    for h in range(LA):
        if h == 2 and jstar == 1:
            seq += [wq_copy(NWQ0 - 1)]
        seq += [k_copy(h), v_copy(h)]
    for c in seq:
        c.start()
        fence()
    acc_s[...] = jnp.zeros_like(acc_s)
    o_s[...] = jnp.zeros_like(o_s)

    def pro_body(it, c):
        hp = it >> 1
        half = it & 1

        @pl.when(it < 2)
        def _():
            x_copy(half).wait()

        @pl.when(half == 0)
        def _():
            wq_copy(hp).wait()

        qproj(hp, half * 4, 4)
        return c

    lax.fori_loop(0, LB, pro_body, 0)

    def a_body(j, c):
        hp = j >> 1
        g = j & 1
        h0 = 2 * j
        jq = j + LB
        hpq = jq >> 1
        gq = jq & 1

        @pl.when(gq == 0)
        def _():
            wq_copy(hpq).wait()

        @pl.when(g == 0)
        def _():
            wo_copy(hp).wait()

        kv_wait(h0)
        kv_wait(h0 + 1)

        @pl.when(jnp.logical_and(gq == 0, hpq + 1 < HP))
        def _():
            wq_copy(jnp.minimum(hpq + 1, HP - 1)).start()

        @pl.when(g == 0)
        def _():
            wo_copy(hp + 1).start()

        kv_start(h0 + LA)
        kv_start(h0 + LA + 1)

        o_prev = o_s[...]
        for i in range(4):
            b = g * 4 + i
            s = (h0 + i // 2) & (NR - 1)
            se, so = scores(hp, b, s, i % 2)
            if i == 0:
                bp = (b + (B - 1)) & (B - 1)
                hpp = jnp.maximum(hp - 1 + g, 0)
            else:
                bp, hpp = b - 1, hp
            outproj(o_prev, hpp, bp)
            qproj(hpq, gq * 4 + i)
            o_prev = pv(se, so, s, i % 2)
        o_s[...] = o_prev
        return c

    lax.fori_loop(0, NAB, a_body, 0)

    def n_body(h, c, last=False, split=False):
        hp = h >> 2
        q4 = h & 3
        b0 = q4 * 2
        s = h & (NR - 1)
        if not last:
            @pl.when(q4 == 0)
            def _():
                wo_copy(hp).wait()
        if split:
            k_copy(h).wait()
        else:
            kv_wait(h)
        if not last:
            @pl.when(jnp.logical_and(q4 == 0, hp + 1 < HP))
            def _():
                wo_copy(jnp.minimum(hp + 1, HP - 1)).start()

            @pl.when(h + LA < NH)
            def _():
                kv_start(jnp.minimum(h + LA, NH - 1))

        o_prev = o_s[...]
        se0, so0 = scores(hp, b0, s, 0)
        se1, so1 = scores(hp, b0 + 1, s, 1)
        if isinstance(h, int):
            bp = (b0 + B - 1) % B
            hpp = hp - 1 if q4 == 0 else hp
        else:
            bp = (b0 + (B - 1)) & (B - 1)
            hpp = jnp.where(q4 == 0, hp - 1, hp)
        outproj(o_prev, hpp, bp, emit=True)
        if split:
            p0 = (_softmax(se0), _softmax(so0))
            p1 = (_softmax(se1), _softmax(so1))
            v_copy(h).wait()
            if last:
                out_copy(0, 6, 0).start()
            o0 = pv_p(*p0, s, 0)
            o1 = pv_p(*p1, s, 1)
        else:
            o0 = pv(se0, so0, s, 0)
            o1 = pv(se1, so1, s, 1)
        outproj(o0, hp, b0, emit=True)
        if last:
            out_copy(6, 1, 1).start()
            outproj(o1, hp, b0 + 1, emit=True)
            out_copy(7, 1, 2).start()
        else:
            o_s[...] = o1
        return c

    lax.fori_loop(H0, NH - NSPLIT, n_body, 0)
    lax.fori_loop(NH - NSPLIT, NH - 1, functools.partial(n_body, split=True), 0)
    n_body(NH - 1, 0, last=True, split=True)
    out_copy(0, 6, 0).wait()
    out_copy(6, 1, 1).wait()
    out_copy(7, 1, 2).wait()


@jax.jit
def pallas_standalone__mha_block_cached__near_ridge_kernel(
    x: jax.Array,
    k_cache: jax.Array,
    v_cache: jax.Array,
    wq: jax.Array,
    wo: jax.Array,
):
    kt = jnp.transpose(k_cache, (0, 1, 3, 2)).reshape(B, HP, PW, SK)
    vt = jnp.transpose(v_cache, (0, 1, 3, 2)).reshape(B, HP, PW, SK)
    x2 = x.reshape(B * SQ, D)
    anyspec = pl.BlockSpec(memory_space=pl.ANY)
    out = pl.pallas_call(
        _kernel,
        in_specs=[anyspec] * 5,
        out_specs=anyspec,
        out_shape=jax.ShapeDtypeStruct((B * SQ, D), BF),
        scratch_shapes=[
            pltpu.VMEM((B * SQ, D), BF),
            pltpu.VMEM((HP, D, PW), BF),
            pltpu.VMEM((HP, PW, D), BF),
            pltpu.VMEM((NR, 2, PW, SK), BF),
            pltpu.VMEM((NR, 2, PW, SK), BF),
            pltpu.VMEM((QR, 2, B * SQ, 256), BF),
            pltpu.VMEM((PW, SQ), BF),
            pltpu.VMEM((B * SQ, D), F32),
            pltpu.VMEM((B * SQ, D), BF),
            pltpu.SemaphoreType.DMA((2,)),
            pltpu.SemaphoreType.DMA((8,)),
            pltpu.SemaphoreType.DMA((2,)),
            pltpu.SemaphoreType.DMA((NR,)),
            pltpu.SemaphoreType.DMA((NR,)),
            pltpu.SemaphoreType.DMA((3,)),
            pltpu.SemaphoreType.REGULAR,
        ],
        compiler_params=pltpu.CompilerParams(
            disable_semaphore_checks=True,
            vmem_limit_bytes=100 * 1024 * 1024),
    )(x2, wq, kt, vt, wo)
    return out.reshape(B, SQ, D)
```
